```python
import os as _os
_os.environ.setdefault("JAX_PLATFORMS", "cpu")
import jax
import jax.numpy as jnp

def _softmax(x, axis=-1):
    return jax.nn.softmax(x, axis=axis)
def _gelu(x):
    return jax.nn.gelu(x, approximate=True)
def _silu(x):
    return jax.nn.silu(x)
def _sigmoid(x):
    return jax.nn.sigmoid(x)
def _layernorm(x, axis=-1, eps=1e-5):
    m = jnp.mean(x, axis=axis, keepdims=True)
    v = jnp.var(x, axis=axis, keepdims=True)
    return (x - m) / jnp.sqrt(v + eps)
def _scatter_add(tgt, idx, src, axis=0):
    return tgt.at[idx].add(src)
def _segment_sum(src, seg, n):
    return jax.ops.segment_sum(src, seg, n)
class _Rng:
    def __init__(self, key):
        self._k = key
    def _next(self):
        self._k, sub = jax.random.split(self._k)
        return sub
    def normal(self, shape):
        return jax.random.normal(self._next(), shape, dtype=jnp.bfloat16)
    def randint(self, lo, hi, shape):
        return jax.random.randint(self._next(), shape, lo, hi, dtype=jnp.int32)
    def uniform(self, shape, lo=0.0, hi=1.0):
        return jax.random.uniform(self._next(), shape, jnp.bfloat16, lo, hi)
    def permutation(self, n):
        return jax.random.permutation(self._next(), n)


kernel_name = 'standalone__layernorm_linear__sampling'

def setup_inputs():
    _rng = _Rng(jax.random.key(int.from_bytes(__import__("os").urandom(4), "little")))
    _w = (lambda a: (lambda t: t.astype(jnp.bfloat16) if jnp.issubdtype(t.dtype, jnp.floating) else t)(jnp.asarray(a)))
    B, S, D = 1024, 32, 576
    return {
        "x": _w((lambda *s: _rng.normal(s) * 0.05)(B, S, D)),
        "g": _w((lambda *s: _rng.normal(s) * 0.05)(D) + 1.0),
        "b": _w((lambda *s: _rng.normal(s) * 0.05)(D)),
        "w": _w((lambda *s: _rng.normal(s) * 0.05)(D, D)),
    }

def reference(x, g, b, w):
    return (_layernorm(x, axis=-1) * g + b) @ w
```

```python
import contextlib
import functools
import jax, jax.numpy as jnp
from jax import lax
from jax.experimental import pallas as pl
from jax.experimental.pallas import tpu as pltpu

F32, BF16, U32 = jnp.float32, jnp.bfloat16, jnp.uint32
T = 128
U = 256
NAMES = "K1t K2t K4t P11 R1l R2l R1r R2r D J P12 P21 K1b K2b K4b P22".split()
IX = {k: i for i, k in enumerate(NAMES)}

def make(segs=((1, 2), (2, 3), (8, 7)), w0=30, ahead=1.0, n1=4, n2=8, flags=None, rp=1, wp=1, cp=None,
         sr=(0.0, 3.9), nr=(0.0, 2.8), wfirst=False, pp=0, p0x=0, scopes=False, refcast=False,
         wgroups=(4, 4, 4, 4, 4, 4, 2, 2, 2, 1), wrows=24, nowrite=False):
    scope = jax.named_scope if scopes else (lambda n: contextlib.nullcontext())
    NP = sum(n * c for n, c in segs)
    groups = []
    p = 0
    for si, (n, c) in enumerate(segs):
        for it in range(c):
            groups.append((si, it, p, n)); p += n
    reads = [(0, 1)]
    rwait = {}
    for si, it, p0, n in groups:
        need = min(p0 + n + 1, NP)
        if n > 1: need += need % 2
        lo = reads[-1][1]
        ids = []
        if lo < need and lo % 2:
            ids.append(len(reads)); reads.append((lo, lo + 1)); lo += 1
        if lo < need:
            ids.append(len(reads)); reads.append((lo, need))
        rwait[si, it] = ids
    writes = {}
    s, sent = 0, 0.0
    for ns in wgroups:
        for r in range(0, 288, wrows):
            p = max(2 * (s + ns), w0 + int(sent - ahead + 1e-6) if sent > ahead else w0)
            writes.setdefault(min(p, NP - 2), []).append((2 * s, 2 * ns, r, wrows, 0, 4 * U))
            sent += ns * wrows / 288
        s += ns
    assert s == NP // 2 - 1
    for r in range(0, 288, 48):
        writes.setdefault(NP - 1, []).append((2 * s, 2, r, 48, 0, 2 * U))

    def kernel(x_hbm, g_hbm, b_hbm, w_hbm, o_hbm, xbuf, obuf, graw, braw, wraw, a_ref, bias, st, pin, stat, op, isem, osem, wsem):
        S, D, B = x_hbm.shape
        NH = D // 2
        HT = T // 2
        def view(ref, lo, hi):
            if hi - lo == 1: return ref.at[lo // 2, :, pl.ds(lo % 2 * 2 * U, 2 * U)]
            assert lo % 2 == 0 and hi % 2 == 0
            return ref.at[pl.ds(lo // 2, (hi - lo) // 2)]
        def cin(i): return pltpu.make_async_copy(view(x_hbm, *reads[i]), view(xbuf, *reads[i]), isem.at[i])
        def cout(h0, nh, r0, nrow, c0, nc):
            v = lambda ref: ref.at[pl.ds(h0, nh), pl.ds(r0, nrow), pl.ds(c0, nc)]
            pltpu.make_async_copy(v(obuf), v(o_hbm), osem).start(priority=wp)
        params = [pltpu.make_async_copy(a, b_, wsem) for a, b_ in ((g_hbm, graw), (b_hbm, braw), (w_hbm, wraw))]
        if not wfirst: cin(0).start(priority=p0x)
        for c in params: c.start(priority=pp)
        if wfirst: cin(0).start(priority=p0x)
        for i in range(1, len(reads)): cin(i).start(priority=rp)

        def prep_weights():
            g = graw[...].astype(F32).reshape(1, D)
            b = braw[...].astype(F32).reshape(1, D)
            lo = lax.broadcasted_iota(jnp.int32, (NH, T), 1) < HT
            sel = lambda u, v: jnp.where(lo, u, v)
            cb = [0.0, 0.0]
            tiles = []
            for k in range(5):
                if k < 4:
                    rows, gk, bk = wraw[pl.ds(k * T, T), :], g[:, k * T:(k + 1) * T], b[:, k * T:(k + 1) * T]
                else:
                    z = wraw[pl.ds(4 * T, HT), :]
                    rows = jnp.concatenate([z, z], axis=0)
                    gk = jnp.concatenate([g[:, 4 * T:]] * 2, axis=1) * (1.0 / 3.0)
                    bk = jnp.concatenate([b[:, 4 * T:]] * 2, axis=1) * 0.5
                wt = rows.astype(F32).T
                halves = wt[:NH], wt[NH:]
                cb = [c + h * bk for c, h in zip(cb, halves)]
                tiles.append([h * gk for h in halves])
            (Pt, Pb), (Qt, Qb), (Xt, Xb), (Yt, Yb), (Zt, Zb) = tiles
            s12, s43 = sel(1.0, 0.5), sel(0.5, 1.0)
            lhs = dict(
                D=Pt + Qb * s12, P11=Qt - Qb * s12, P22=Pb * s12 - Pt,
                J=Xt + Yb * s43, P12=Yt - Yb * s43, P21=Xb * s43 - Xt,
                R1l=sel(Qb, Xt), R1r=sel(Pt, Yb), R2l=sel(Xt, Qb * 0.5), R2r=sel(Yb * 0.5, Pt),
                K1t=sel(-(Pt + Qt), Xt + Yt), K1b=sel(Pb + Qb, -(Xb + Yb)),
                K2t=sel(Zt, -(Pt + Qt)), K2b=sel(Zb, (Pb + Qb) * 0.5),
                K4t=sel(Xt + Yt, -Zt), K4b=sel((Xb + Yb) * -0.5, -Zb))
            for k in NAMES:
                a_ref[IX[k]] = pltpu.bitcast(lhs[k].astype(BF16), U32)
            for h in range(2):
                bias[h] = jnp.broadcast_to(jnp.sum(cb[h], axis=1, keepdims=True), (NH, T))

        st[0, :8, :] = jnp.zeros((8, T), F32)

        def gate(slot, v, anchor):
            if anchor is not None:
                pin[slot] = jnp.concatenate([anchor, anchor], axis=1)
            pin[slot] = v
            return pin[slot]

        def stats(s, col, h):
            def sweep(f, n):
                acc = None
                rows = list(range(0, D, 8))
                per = len(rows) // n
                for c in range(n):
                    anchor = yield
                    for r in rows[c * per:(c + 1) * per]:
                        v = f(xbuf[s, pl.ds(r, 8), col].astype(F32))
                        acc = v if acc is None else acc + v
                    acc = gate(0, acc, anchor)
                return jnp.sum(acc, axis=0, keepdims=True) * (1.0 / D)
            m = jnp.broadcast_to((yield from sweep(lambda v: v, n1)), (8, U))
            stat[h, 0] = m
            def sq(v):
                d = v - m
                return d * d
            stat[h, 1] = jnp.broadcast_to(lax.rsqrt((yield from sweep(sq, n2)) + 1e-5), (8, U))
            yield

        n3 = 20
        def norm(s, col, h):
            m8 = None
            def put(name, upper, r, v): op[h, IX[name], pl.ds(upper * HT + r, 16), :] = v.astype(BF16)
            for r in range(0, HT, 16):
                for blk in range(5):
                    anchor = yield
                    if m8 is None: m8, rs = stat[h, 0], stat[h, 1][:1]
                    m = gate(1, m8, anchor)[:1]
                    def xn(row):
                        v = (xbuf[s, pl.ds(row, 16), col].astype(F32) - m) * rs
                        return v[:, :T], v[:, T:]
                    if blk == 4:
                        zl, zr = xn(4 * T + r)
                        t = zl + zr
                        u2, u4 = t + zl, t + zr
                        put("K2t", 0, r, u2); put("K2b", 0, r, u2); put("K4t", 1, r, u4); put("K4b", 1, r, u4)
                        continue
                    swap, upper = divmod(blk, 2)
                    row = swap * 2 * T + upper * HT + r
                    (b11, b12), (b21, b22) = xn(row), xn(row + T)
                    if swap: b11, b12, b21, b22 = b12, b11, b22, b21
                    twice = swap != upper
                    c22, c12 = (b22 + b22, b12 + b12) if twice else (b22, b12)
                    names = (("D P11 P22 R1l R1r K1t K1b", "D P11 P22 R2l R2r K2t K2b"), ("J P12 P21 R2r R2l K4t K4b", "J P12 P21 R1r R1l K1t K1b"))[swap][upper]
                    for name, v in zip(names.split(), (b11 + c22, b21 + c22, b11 + c12, b21 - b11, b12 - b22, b22, b11)):
                        put(name, upper, r, v)
            yield

        def steps(gen, rng, n):
            next(gen)
            return [(rng[0] + (rng[1] - rng[0]) * c / max(n - 1, 1), gen.send) for c in range(n)]

        def unit(s, col, h, tasks, flush):
            tasks = sorted(tasks, key=lambda t: t[0])
            def rhs(i): return pltpu.bitcast(op.bitcast(U32)[h, i], BF16) if refcast else op[h, i]
            def prods(r):
                return [jnp.dot(pltpu.bitcast(a_ref[i], BF16), rhs(i), preferred_element_type=F32) for i in range(4 * r, 4 * r + 4)]
            def done(r, v):
                while tasks and tasks[0][0] < r + 1:
                    pos, fn = tasks.pop(0)
                    row = int((pos - r) * NH) // 8 * 8
                    fn(v[row:row + 8])
            def out(half, c1, c2):
                obuf[2 * s + half, :, col] = jnp.concatenate([c1, c2], axis=1).astype(BF16)
                flush(half)
            k1, k2, k4, p11 = prods(0)
            e, bt = k1 + k2 + k4, bias[0]
            st[0] = (bt + p11) + (e + k2); st[1] = (bt - k4) - e
            done(0, p11)
            r1l, r2l, r1r, r2r = prods(1)
            fl, fr, bb = r1l + r2l, r1r + r2r, bias[1]
            st[2] = st[0] + fl; st[3] = st[1] + fr; st[4] = (bb + r2l) + fl; st[5] = (bb + r2r) + fr
            done(1, r2r)
            d, j, p12, p21 = prods(2)
            out(0, st[2] + d, (st[3] + j) + p12)
            st[6] = (st[4] + j) + p21; st[7] = st[5] + d
            done(2, p21)
            k1, k2, k4, p22 = prods(3)
            e = k1 + k2 + k4
            out(1, (st[6] + k2) + e, (st[7] + p22) - (e + k4))
            done(3, p22)
            assert not tasks

        def pair(cur, nxt, flush):
            (s, ca, cb), (s2, ca2, cb2) = cur, nxt
            unit(s, ca, 0, steps(norm(s, cb, 1), nr, n3) + steps(stats(s2, ca2, 0), sr, n1 + n2), functools.partial(flush, 0))
            unit(s, cb, 1, steps(norm(s2, ca2, 0), nr, n3) + steps(stats(s2, cb2, 1), sr, n1 + n2), functools.partial(flush, 1))

        def first_ln():
            with scope("wait_x0"): cin(0).wait()
            for _, fn in steps(stats(0, pl.ds(0, U), 0), (0, 0), n1 + n2) + steps(norm(0, pl.ds(0, U), 0), (0, 0), n3) + steps(stats(0, pl.ds(U, U), 1), (0, 0), n1 + n2):
                fn(None)
        if not wfirst: first_ln()
        with scope("wait_w"):
            for c in params: c.wait()
        with scope("prep_w"): prep_weights()
        if wfirst: first_ln()

        def tail(h, half): cout(2 * S - 2 + half, 1, 0, NH, B - 2 * U + h * U, U)

        p0 = 0
        for si, (n, cnt) in enumerate(segs):
            def body(it, _, si=si, n=n, cnt=cnt, p0=p0):
                with scope(f"wait_in{si}"):
                    for k in range(cnt):
                        for i in rwait[si, k]:
                            pl.when(it == k)(cin(i).wait)
                def loc(j):
                    if n % 2 == 0 and p0 % 2 == 0:
                        s, half = it * (n // 2) + (p0 + j) // 2, j % 2
                        if j == n: s = jnp.minimum(s, S - 1)
                        return s, pl.ds(half * 2 * U, U), pl.ds(half * 2 * U + U, U)
                    p = jnp.minimum(p0 + it * n + j, NP - 1)
                    c = (p % 2) * 2 * U
                    return p // 2, pl.ds(pl.multiple_of(c, U), U), pl.ds(pl.multiple_of(c + U, U), U)
                for j in range(n):
                    for k in range(cnt):
                        ws = writes.get(p0 + k * n + j)
                        if ws and not nowrite:
                            @pl.when(it == k)
                            def _():
                                for wr in ws: cout(*wr)
                    def flush(h, half, j=j):
                        if p0 + cnt * n == NP and j == n - 1 and (h, half) != (1, 1) and not nowrite:
                            pl.when(it == cnt - 1)(functools.partial(tail, h, half))
                    pair(loc(j), loc(j + 1), flush)
            with scope(f"seg{si}"): lax.fori_loop(0, cnt, body, None)
            p0 += n * cnt
        if not nowrite:
            tail(1, 1)
            with scope("wait_out"): pltpu.make_async_copy(obuf, o_hbm, osem).wait()

    def fn(x, g, b, w):
        B, S, D = x.shape
        xt = jnp.transpose(x, (1, 2, 0))
        out = pl.pallas_call(
            kernel,
            in_specs=[pl.BlockSpec(memory_space=pl.ANY)] * 4,
            out_specs=pl.BlockSpec(memory_space=pl.ANY),
            out_shape=jax.ShapeDtypeStruct((2 * S, D // 2, B), x.dtype),
            scratch_shapes=[pltpu.VMEM((S, D, B), BF16), pltpu.VMEM((2 * S, D // 2, B), BF16), pltpu.VMEM((D,), BF16), pltpu.VMEM((D,), BF16), pltpu.VMEM((D, D), BF16),
                            pltpu.VMEM((16, D // 4, T), U32), pltpu.VMEM((2, D // 2, T), F32), pltpu.VMEM((8, D // 2, T), F32), pltpu.VMEM((2, 8, U), F32), pltpu.VMEM((2, 2, 8, U), F32),
                            pltpu.VMEM((2, 16, T, T), BF16),
                            pltpu.SemaphoreType.DMA((len(reads),)), pltpu.SemaphoreType.DMA(()), pltpu.SemaphoreType.DMA(())],
            compiler_params=pltpu.CompilerParams(vmem_limit_bytes=110 * 2**20, flags=flags, **(cp or {})),
        )(xt, g, b, w)
        return jnp.transpose(out.reshape(S, D, B), (2, 0, 1))
    return fn


@jax.jit
def pallas_standalone__layernorm_linear__sampling_kernel(x, g, b, w):
    return make()(x, g, b, w)
```

```python
import functools

import jax
import jax.numpy as jnp
from jax import lax
import jax.experimental.pallas as pl
import jax.experimental.pallas.tpu as pltpu

F32, BF16, U32 = jnp.float32, jnp.bfloat16, jnp.uint32
EPS = 1e-5
T = 128
HT = T // 2
UNIT = 2 * T
PAIR = 2 * UNIT
PAIRS_PER_STEP = 16

PRODUCTS = {
    "K1t": ((0, 5), (3, 5)), "K2t": ((4, 0), (1, 5)), "K4t": ((2, 5), (4, 1)), "P11": ((0, 1), (1, 1)),
    "R1l": ((0, 3), (3, 4)), "R2l": ((2, 4), (1, 3)), "R1r": ((0, 4), (3, 3)), "R2r": ((2, 3), (1, 4)),
    "D": ((0, 0), (1, 0)), "J": ((2, 0), (3, 0)), "P12": ((2, 1), (3, 1)), "P21": ((2, 2), (3, 2)),
    "K1b": ((0, 6), (3, 6)), "K2b": ((4, 0), (1, 6)), "K4b": ((2, 6), (4, 1)), "P22": ((0, 2), (1, 2)),
}

MEAN_CHUNKS, VAR_CHUNKS, STAT_SPAN = 8, 12, (0.1, 3.9)
NORM_CHUNKS, NORM_SPAN = 20, (0.15, 2.9)

READ_EDGES = (2, 4, 6, 10, 18, 34, 64)
WRITE_GROUPS, WRITE_ROWS, FIRST_WRITE = (8, 4, 4, 4, 4, 2, 2, 1), 24, 62


def _pack(v):
    return pltpu.bitcast(v.astype(BF16), U32)


def _write_plan(n_units, half_rows):
    plan, slab, sent = {}, 0, 0
    for n in WRITE_GROUPS:
        for r in range(0, half_rows, WRITE_ROWS):
            unit = max(4 * (slab + n), FIRST_WRITE + max(2 * sent // half_rows - 2, 0))
            plan.setdefault(min(unit, n_units - 1), []).append((2 * slab, 2 * n, r, WRITE_ROWS, 0, 2 * PAIR))
            sent += n * WRITE_ROWS
        slab += n
    for p in range(2 * slab, n_units // 2 - 1):
        for half in range(2):
            plan.setdefault(2 * p + 2, []).append((p // 2 * 2 + half, 1, 0, half_rows, p % 2 * PAIR, PAIR))
    return plan


def _body(x_hbm, g_hbm, b_hbm, w_hbm, o_hbm,
          x_buf, o_buf, g_buf, b_buf, w_buf, wt, lhs, bias, terms, part, stat, pin,
          out_sem, param_sems, in_sems):
    S, D, B = x_hbm.shape
    NH = D // 2
    n_pairs = S * B // PAIR
    n_steps = n_pairs // PAIRS_PER_STEP
    writes = _write_plan(2 * n_pairs, NH)

    def read_pair(p):
        def view(ref):
            return ref.at[0, :, pl.ds(pl.multiple_of(p * PAIR, PAIR), PAIR)]
        return pltpu.make_async_copy(view(x_hbm), view(x_buf), in_sems.at[p])

    def read_slabs(i):
        slabs = pl.ds(READ_EDGES[i] // 2, (READ_EDGES[i + 1] - READ_EDGES[i]) // 2)
        return pltpu.make_async_copy(x_hbm.at[slabs], x_buf.at[slabs], in_sems.at[2 + i])

    def write(half0, n_halves, row0, n_rows, col0, n_cols):
        def view(ref):
            return ref.at[pl.ds(half0, n_halves), pl.ds(row0, n_rows), pl.ds(col0, n_cols)]
        pltpu.make_async_copy(view(o_buf), view(o_hbm), out_sem).start()

    def prepare_weights():
        for k in range(4):
            wt[k] = w_buf[pl.ds(k * T, T), :].T.astype(F32)
        ninth = w_buf[pl.ds(4 * T, HT), :]
        wt[4] = jnp.concatenate([ninth, ninth], axis=0).T.astype(F32)

        def lane_tiles(ref, ninth_scale):
            v = ref[...].astype(F32).reshape(1, D)
            last = jnp.concatenate([v[:, 4 * T:]] * 2, axis=1) * ninth_scale
            return [v[:, k * T:(k + 1) * T] for k in range(4)] + [last]

        g, b = lane_tiles(g_buf, 1.0 / 3.0), lane_tiles(b_buf, 0.5)
        join = functools.partial(jnp.where, lax.broadcasted_iota(jnp.int32, (16, T), 1) < HT)
        s01, s23 = join(1.0, 0.5), join(0.5, 1.0)
        for r in range(0, NH, 16):
            halves = []
            for half in range(2):
                ws = [wt[k, pl.ds(half * NH + r, 16), :] for k in range(5)]
                bw = functools.reduce(jnp.add, [u * v for u, v in zip(ws, b)])
                bias[half, pl.ds(r, 16), :] = jnp.broadcast_to(jnp.sum(bw, axis=1, keepdims=True), (16, T))
                halves.append([u * v for u, v in zip(ws, g)])
            (pt, qt, xt, yt, zt), (pb, qb, xb, yb, zb) = halves
            qs, ys = qb * s01, yb * s23
            pqt, xyt, pqb, xyb = -(pt + qt), xt + yt, (pb + qb) * s01, (xb + yb) * -s23
            tiles = dict(
                D=pt + qs, P11=qt - qs, P22=pb * s01 - pt,
                J=xt + ys, P12=yt - ys, P21=xb * s23 - xt,
                R1l=join(qs, xt), R1r=join(pt, ys), R2l=join(xt, qs), R2r=join(ys, pt),
                K1t=join(pqt, xyt), K1b=join(pqb, xyb),
                K2t=join(zt, pqt), K2b=join(zb, pqb), K4t=join(xyt, -zt), K4b=join(xyb, -zb))
            lhs[:, pl.ds(r // 2, 8), :] = _pack(jnp.stack([tiles[name] for name in PRODUCTS]))

    def after(slot, value, marker):
        if marker is not None:
            pin[slot] = jnp.concatenate([marker, marker], axis=1)
        pin[slot] = value
        return pin[slot]

    def statistics(s, cols, h, marker):
        def column_mean(f, first, chunks):
            acc, rows = None, D // chunks
            for c in range(chunks):
                v = f(x_buf[s, pl.ds(c * rows, rows), cols].astype(F32))
                v = jnp.sum(v.reshape(rows // 8, 8, UNIT), axis=0)
                acc = after(0, v if acc is None else acc + v,
                            marker(STAT_SPAN, first + c, MEAN_CHUNKS + VAR_CHUNKS))
            return jnp.sum(acc, axis=0, keepdims=True) * (1.0 / D)

        mean = column_mean(lambda v: v, 0, MEAN_CHUNKS)
        var = column_mean(lambda v: jnp.square(v - mean), MEAN_CHUNKS, VAR_CHUNKS)
        stat[h, 0] = jnp.broadcast_to(mean, (8, UNIT))
        stat[h, 1] = jnp.broadcast_to(lax.rsqrt(var + EPS), (8, UNIT))

    def normalize(s, cols, h, marker):
        mean8, rstd = stat[h, 0], stat[h, 1][:1]
        for c in range(NORM_CHUNKS):
            r, step = c // 5 * 16, c % 5
            mean = after(1, mean8, marker(NORM_SPAN, c, NORM_CHUNKS))[:1]

            def xhat(row):
                v = (x_buf[s, pl.ds(row + r, 16), cols].astype(F32) - mean) * rstd
                return v[:, :T], v[:, T:]

            if step == 4:
                left, right = xhat(4 * T)
                both = left + right
                vals = [both + left, both + right]
            else:
                row = step // 2 * 2 * T + step % 2 * HT
                (b11, b12), (b21, b22) = xhat(row), xhat(row + T)
                if step in (2, 3):
                    b11, b12, b21, b22 = b12, b11, b22, b21
                c12, c22 = (b12 + b12, b22 + b22) if step in (1, 2) else (b12, b22)
                vals = [b11 + c22, b21 + c22, b11 + c12, b21 - b11, b12 - b22, b22, b11]
            terms[h, pl.ds(7 * step, len(vals)), pl.ds(r // 2, 8), :] = _pack(jnp.stack(vals))

    def multiply(s, cols, h, on_stored):
        sources = list(PRODUCTS.values())

        def products(rnd):
            out = []
            for i in range(4 * rnd, 4 * rnd + 4):
                tile = jnp.concatenate([terms[h, 7 * step + term] for step, term in sources[i]], axis=0)
                out.append(jnp.dot(pltpu.bitcast(lhs[i], BF16), pltpu.bitcast(tile, BF16),
                                   preferred_element_type=F32))
            return out

        def store(half, left, right):
            o_buf[2 * s + half, :, cols] = jnp.concatenate([left, right], axis=1).astype(o_buf.dtype)
            on_stored(h, half)

        k1, k2, k4, p11 = products(0)
        e, top = k1 + k2 + k4, bias[0]
        part[0] = (top + p11) + (e + k2)
        part[1] = (top - k4) - e
        r1l, r2l, r1r, r2r = products(1)
        fl, fr, bottom = r1l + r2l, r1r + r2r, bias[1]
        part[2] = part[0] + fl
        part[3] = part[1] + fr
        part[4] = (bottom + r2l) + fl
        part[5] = (bottom + r2r) + fr
        d, j, p12, p21 = products(2)
        store(0, part[2] + d, (part[3] + j) + p12)
        part[6] = (part[4] + j) + p21
        part[7] = part[5] + d
        k1, k2, k4, p22 = products(3)
        e = k1 + k2 + k4
        store(1, (part[6] + k2) + e, (part[7] + p22) - (e + k4))

        def marker(span, i, count):
            pos = span[0] + (span[1] - span[0]) * i / (count - 1)
            row = int(pos % 1 * NH) // 8 * 8
            return (p11, r2r, p21, p22)[int(pos)][row:row + 8]
        return marker

    params = [pltpu.make_async_copy(src, dst, param_sems.at[i])
              for i, (src, dst) in enumerate(((w_hbm, w_buf), (g_hbm, g_buf), (b_hbm, b_buf)))]
    for copy in params:
        copy.start()
    lax.fori_loop(0, 2, lambda p, _: read_pair(p).start(), None)
    for copy in params:
        copy.wait()
    for i in range(len(READ_EDGES) - 1):
        read_slabs(i).start()
    part[0, :8, :] = jnp.zeros((8, T), F32)
    prepare_weights()

    def unpaced(*_):
        return None

    def first_statistics(h, _):
        pl.when(h == 0)(read_pair(0).wait)
        statistics(0, pl.ds(pl.multiple_of(h * UNIT, UNIT), UNIT), h, unpaced)

    lax.fori_loop(0, 2, first_statistics, None)
    normalize(0, pl.ds(0, UNIT), 0, unpaced)

    def step(it, _):
        n = PAIRS_PER_STEP

        def locate(j):
            s, col = it * (n // 2) + j // 2, j % 2 * PAIR
            return (jnp.minimum(s, S - 1) if j == n else s), pl.ds(col, UNIT), pl.ds(col + UNIT, UNIT)

        def start_writes(unit):
            for k in range(n_steps):
                for piece in writes.get(2 * k * n + unit, ()):
                    pl.when(it == k)(functools.partial(write, *piece))

        wt[0, :8, :] = jnp.zeros((8, T), F32)
        for j in range(n):
            def on_stored(h, half):
                if j == n - 1:
                    piece = (2 * S - 2 + half, 1, 0, NH, PAIR + h * UNIT, UNIT)
                    pl.when(it == n_steps - 1)(functools.partial(write, *piece))

            (s, first, second), (s_next, first_next, second_next) = locate(j), locate(j + 1)
            start_writes(2 * j)
            marker = multiply(s, first, 0, on_stored)
            if j == 0:
                pl.when(it == 0)(read_pair(1).wait)
            for i, edge in enumerate(READ_EDGES[:-1]):
                if (edge - 1) % n == j:
                    pl.when(it == (edge - 1) // n)(read_slabs(i).wait)
            normalize(s, second, 1, marker)
            statistics(s_next, first_next, 0, marker)
            start_writes(2 * j + 1)
            marker = multiply(s, second, 1, on_stored)
            normalize(s_next, first_next, 0, marker)
            statistics(s_next, second_next, 1, marker)

    lax.fori_loop(0, n_steps, step, None)
    pltpu.make_async_copy(o_buf, o_hbm, out_sem).wait()


def _kernel(*refs):
    pl.run_scoped(functools.partial(_body, *refs),
                  pltpu.SemaphoreType.DMA((3,)), pltpu.SemaphoreType.DMA((len(READ_EDGES) + 1,)))


@jax.jit
def pallas_standalone__layernorm_linear__sampling_kernel(
    x: jax.Array,
    g: jax.Array,
    b: jax.Array,
    w: jax.Array,
):
    B, S, D = x.shape
    assert (B, S, D) == (2 * PAIR, READ_EDGES[-1] // 2, 9 * HT)
    out = pl.pallas_call(
        _kernel,
        in_specs=[pl.BlockSpec(memory_space=pl.ANY)] * 4,
        out_specs=pl.BlockSpec(memory_space=pl.ANY),
        out_shape=jax.ShapeDtypeStruct((2 * S, D // 2, B), x.dtype),
        scratch_shapes=[
            pltpu.VMEM((S, D, B), x.dtype),
            pltpu.VMEM((2 * S, D // 2, B), x.dtype),
            pltpu.VMEM((D,), g.dtype),
            pltpu.VMEM((D,), b.dtype),
            pltpu.VMEM((D, D), w.dtype),
            pltpu.VMEM((5, D, T), F32),
            pltpu.VMEM((16, D // 4, T), U32),
            pltpu.VMEM((2, D // 2, T), F32),
            pltpu.VMEM((2, 30, HT // 2, T), U32),
            pltpu.VMEM((8, D // 2, T), F32),
            pltpu.VMEM((2, 2, 8, UNIT), F32),
            pltpu.VMEM((2, 8, UNIT), F32),
            pltpu.SemaphoreType.DMA(()),
        ],
        compiler_params=pltpu.CompilerParams(
            vmem_limit_bytes=100 * 2**20,
            flags={"XLA_TPU_RESCHEDULE_DMA_DONES": True},
        ),
    )(jnp.transpose(x, (1, 2, 0)), g, b, w)
    return jnp.transpose(out.reshape(S, D, B), (2, 0, 1))
```

```python
import functools

import jax
import jax.numpy as jnp
from jax import lax
import jax.experimental.pallas as pl
import jax.experimental.pallas.tpu as pltpu

F32, BF16, U32 = jnp.float32, jnp.bfloat16, jnp.uint32
EPS = 1e-5
T = 128
HT = T // 2
UNIT = 2 * T
PAIR = 2 * UNIT
PAIRS_PER_STEP = 16

PRODUCTS = {
    "K1t": ((0, 5), (3, 5)), "K2t": ((4, 0), (1, 5)), "K4t": ((2, 5), (4, 1)), "P11": ((0, 1), (1, 1)),
    "R1l": ((0, 3), (3, 4)), "R2l": ((2, 4), (1, 3)), "R1r": ((0, 4), (3, 3)), "R2r": ((2, 3), (1, 4)),
    "D": ((0, 0), (1, 0)), "J": ((2, 0), (3, 0)), "P12": ((2, 1), (3, 1)), "P21": ((2, 2), (3, 2)),
    "K1b": ((0, 6), (3, 6)), "K2b": ((4, 0), (1, 6)), "K4b": ((2, 6), (4, 1)), "P22": ((0, 2), (1, 2)),
}

MEAN_CHUNKS, VAR_CHUNKS, STAT_SPAN = 8, 12, (0.1, 3.9)
NORM_CHUNKS, NORM_SPAN = 20, (0.15, 2.9)

READ_EDGES = (4, 6, 10, 18, 34, 64)
WRITE_GROUPS, WRITE_ROWS, FIRST_WRITE = (8, 4, 4, 4, 4, 2, 2, 1, 1), 24, 62


def _pack(v):
    return pltpu.bitcast(v.astype(BF16), U32)


def _write_plan(n_units, half_rows):
    plan, slab, sent = {}, 0, 0
    for n in WRITE_GROUPS:
        for r in range(0, half_rows, WRITE_ROWS):
            unit = max(4 * (slab + n), FIRST_WRITE + max(2 * sent // half_rows - 2, 0))
            plan.setdefault(min(unit, n_units - 1), []).append((2 * slab, 2 * n, r, WRITE_ROWS, 0, 2 * PAIR))
            sent += n * WRITE_ROWS
        slab += n
    for p in range(2 * slab, n_units // 2 - 1):
        for half in range(2):
            plan.setdefault(2 * p + 2, []).append((p // 2 * 2 + half, 1, 0, half_rows, p % 2 * PAIR, PAIR))
    return plan


def _body(x_hbm, g_hbm, b_hbm, w_hbm, o_hbm,
          x_buf, o_buf, g_buf, b_buf, w_buf, wt, lhs, bias, terms, part, stat, pin,
          out_sem, param_sems, in_sems):
    S, D, B = x_hbm.shape
    NH = D // 2
    n_pairs = S * B // PAIR
    n_steps = n_pairs // PAIRS_PER_STEP
    writes = _write_plan(2 * n_pairs, NH)

    def read_pair(p):
        def view(ref):
            return ref.at[p // 2, :, pl.ds(pl.multiple_of(p % 2 * PAIR, PAIR), PAIR)]
        return pltpu.make_async_copy(view(x_hbm), view(x_buf), in_sems.at[p])

    def read_slabs(i):
        slabs = pl.ds(READ_EDGES[i] // 2, (READ_EDGES[i + 1] - READ_EDGES[i]) // 2)
        return pltpu.make_async_copy(x_hbm.at[slabs], x_buf.at[slabs], in_sems.at[READ_EDGES[0] + i])

    def write(half0, n_halves, row0, n_rows, col0, n_cols):
        def view(ref):
            return ref.at[pl.ds(half0, n_halves), pl.ds(row0, n_rows), pl.ds(col0, n_cols)]
        pltpu.make_async_copy(view(o_buf), view(o_hbm), out_sem).start()

    def prepare_weights():
        for k in range(4):
            wt[k] = w_buf[pl.ds(k * T, T), :].T.astype(F32)
        ninth = w_buf[pl.ds(4 * T, HT), :]
        wt[4] = jnp.concatenate([ninth, ninth], axis=0).T.astype(F32)

        def lane_tiles(ref, ninth_scale):
            v = ref[...].astype(F32).reshape(1, D)
            last = jnp.concatenate([v[:, 4 * T:]] * 2, axis=1) * ninth_scale
            return [v[:, k * T:(k + 1) * T] for k in range(4)] + [last]

        g, b = lane_tiles(g_buf, 1.0 / 3.0), lane_tiles(b_buf, 0.5)
        join = functools.partial(jnp.where, lax.broadcasted_iota(jnp.int32, (16, T), 1) < HT)
        s01, s23 = join(1.0, 0.5), join(0.5, 1.0)
        for r in range(0, NH, 16):
            halves = []
            for half in range(2):
                ws = [wt[k, pl.ds(half * NH + r, 16), :] for k in range(5)]
                bias[half, pl.ds(r, 16), :] = functools.reduce(jnp.add, [u * v for u, v in zip(ws, b)])
                halves.append([u * v for u, v in zip(ws, g)])
            (pt, qt, xt, yt, zt), (pb, qb, xb, yb, zb) = halves
            qs, ys = qb * s01, yb * s23
            pqt, xyt, pqb, xyb = -(pt + qt), xt + yt, (pb + qb) * s01, (xb + yb) * -s23
            tiles = dict(
                D=pt + qs, P11=qt - qs, P22=pb * s01 - pt,
                J=xt + ys, P12=yt - ys, P21=xb * s23 - xt,
                R1l=join(qs, xt), R1r=join(pt, ys), R2l=join(xt, qs), R2r=join(ys, pt),
                K1t=join(pqt, xyt), K1b=join(pqb, xyb),
                K2t=join(zt, pqt), K2b=join(zb, pqb), K4t=join(xyt, -zt), K4b=join(xyb, -zb))
            lhs[:, pl.ds(r // 2, 8), :] = _pack(jnp.stack([tiles[name] for name in PRODUCTS]))

    def after(slot, value, marker):
        if marker is not None:
            pin[slot] = jnp.concatenate([marker, marker], axis=1)
        pin[slot] = value
        return pin[slot]

    def statistics(s, cols, h, marker):
        def column_mean(f, first, chunks):
            acc, rows = None, D // chunks
            for c in range(chunks):
                v = f(x_buf[s, pl.ds(c * rows, rows), cols].astype(F32))
                v = jnp.sum(v.reshape(rows // 8, 8, UNIT), axis=0)
                acc = after(0, v if acc is None else acc + v,
                            marker(STAT_SPAN, first + c, MEAN_CHUNKS + VAR_CHUNKS))
            return jnp.sum(acc, axis=0, keepdims=True) * (1.0 / D)

        mean = column_mean(lambda v: v, 0, MEAN_CHUNKS)
        var = column_mean(lambda v: jnp.square(v - mean), MEAN_CHUNKS, VAR_CHUNKS)
        stat[h, 0] = jnp.broadcast_to(mean, (8, UNIT))
        stat[h, 1] = jnp.broadcast_to(lax.rsqrt(var + EPS), (8, UNIT))

    def normalize(s, cols, h, marker):
        mean8, rstd = stat[h, 0], stat[h, 1][:1]
        for c in range(NORM_CHUNKS):
            r, step = c // 5 * 16, c % 5
            mean = after(1, mean8, marker(NORM_SPAN, c, NORM_CHUNKS))[:1]

            def xhat(row):
                v = (x_buf[s, pl.ds(row + r, 16), cols].astype(F32) - mean) * rstd
                return v[:, :T], v[:, T:]

            if step == 4:
                left, right = xhat(4 * T)
                both = left + right
                vals = [both + left, both + right]
            else:
                row = step // 2 * 2 * T + step % 2 * HT
                (b11, b12), (b21, b22) = xhat(row), xhat(row + T)
                if step in (2, 3):
                    b11, b12, b21, b22 = b12, b11, b22, b21
                c12, c22 = (b12 + b12, b22 + b22) if step in (1, 2) else (b12, b22)
                vals = [b11 + c22, b21 + c22, b11 + c12, b21 - b11, b12 - b22, b22, b11]
            terms[h, pl.ds(7 * step, len(vals)), pl.ds(r // 2, 8), :] = _pack(jnp.stack(vals))

    def multiply(s, cols, h, on_stored):
        sources = list(PRODUCTS.values())

        def products(rnd):
            out = []
            for i in range(4 * rnd, 4 * rnd + 4):
                tile = jnp.concatenate([terms[h, 7 * step + term] for step, term in sources[i]], axis=0)
                out.append(jnp.dot(pltpu.bitcast(lhs[i], BF16), pltpu.bitcast(tile, BF16),
                                   preferred_element_type=F32))
            return out

        def store(half, left, right):
            o_buf[2 * s + half, :, cols] = jnp.concatenate([left, right], axis=1).astype(o_buf.dtype)
            on_stored(h, half)

        k1, k2, k4, p11 = products(0)
        e, top = k1 + k2 + k4, bias[0]
        part[0] = (top + p11) + (e + k2)
        part[1] = (top - k4) - e
        r1l, r2l, r1r, r2r = products(1)
        fl, fr, bottom = r1l + r2l, r1r + r2r, bias[1]
        part[2] = part[0] + fl
        part[3] = part[1] + fr
        part[4] = (bottom + r2l) + fl
        part[5] = (bottom + r2r) + fr
        d, j, p12, p21 = products(2)
        store(0, part[2] + d, (part[3] + j) + p12)
        part[6] = (part[4] + j) + p21
        part[7] = part[5] + d
        k1, k2, k4, p22 = products(3)
        e = k1 + k2 + k4
        store(1, (part[6] + k2) + e, (part[7] + p22) - (e + k4))

        def marker(span, i, count):
            pos = span[0] + (span[1] - span[0]) * i / (count - 1)
            row = int(pos % 1 * NH) // 8 * 8
            return (p11, r2r, p21, p22)[int(pos)][row:row + 8]
        return marker

    params = [pltpu.make_async_copy(src, dst, param_sems.at[i])
              for i, (src, dst) in enumerate(((w_hbm, w_buf), (g_hbm, g_buf), (b_hbm, b_buf)))]
    for copy in params:
        copy.start()
    lax.fori_loop(0, READ_EDGES[0], lambda p, _: read_pair(p).start(), None)
    for copy in params:
        copy.wait()
    for i in range(len(READ_EDGES) - 1):
        read_slabs(i).start()
    part[0, :8, :] = jnp.zeros((8, T), F32)
    prepare_weights()

    def unpaced(*_):
        return None

    def first_statistics(h, _):
        pl.when(h == 0)(read_pair(0).wait)
        statistics(0, pl.ds(pl.multiple_of(h * UNIT, UNIT), UNIT), h, unpaced)
        bias[h] = jnp.broadcast_to(jnp.sum(bias[h], axis=1, keepdims=True), (NH, T))

    lax.fori_loop(0, 2, first_statistics, None)
    normalize(0, pl.ds(0, UNIT), 0, unpaced)

    def step(it, _):
        n = PAIRS_PER_STEP

        def locate(j):
            s, col = it * (n // 2) + j // 2, j % 2 * PAIR
            return (jnp.minimum(s, S - 1) if j == n else s), pl.ds(col, UNIT), pl.ds(col + UNIT, UNIT)

        def start_writes(unit):
            for k in range(n_steps):
                for piece in writes.get(2 * k * n + unit, ()):
                    pl.when(it == k)(functools.partial(write, *piece))

        wt[0, :8, :] = jnp.zeros((8, T), F32)
        for j in range(n):
            def on_stored(h, half):
                if j == n - 1:
                    piece = (2 * S - 2 + half, 1, 0, NH, PAIR + h * UNIT, UNIT)
                    pl.when(it == n_steps - 1)(functools.partial(write, *piece))

            (s, first, second), (s_next, first_next, second_next) = locate(j), locate(j + 1)
            start_writes(2 * j)
            marker = multiply(s, first, 0, on_stored)
            if j + 1 < READ_EDGES[0]:
                pl.when(it == 0)(read_pair(j + 1).wait)
            for i, edge in enumerate(READ_EDGES[:-1]):
                if (edge - 1) % n == j:
                    pl.when(it == (edge - 1) // n)(read_slabs(i).wait)
            normalize(s, second, 1, marker)
            statistics(s_next, first_next, 0, marker)
            start_writes(2 * j + 1)
            marker = multiply(s, second, 1, on_stored)
            normalize(s_next, first_next, 0, marker)
            statistics(s_next, second_next, 1, marker)

    lax.fori_loop(0, n_steps, step, None)
    pltpu.make_async_copy(o_buf, o_hbm, out_sem).wait()


def _kernel(*refs):
    pl.run_scoped(functools.partial(_body, *refs),
                  pltpu.SemaphoreType.DMA((3,)),
                  pltpu.SemaphoreType.DMA((READ_EDGES[0] + len(READ_EDGES) - 1,)))


@jax.jit
def pallas_standalone__layernorm_linear__sampling_kernel(
    x: jax.Array,
    g: jax.Array,
    b: jax.Array,
    w: jax.Array,
):
    B, S, D = x.shape
    assert (B, S, D) == (2 * PAIR, READ_EDGES[-1] // 2, 9 * HT)
    out = pl.pallas_call(
        _kernel,
        in_specs=[pl.BlockSpec(memory_space=pl.ANY)] * 4,
        out_specs=pl.BlockSpec(memory_space=pl.ANY),
        out_shape=jax.ShapeDtypeStruct((2 * S, D // 2, B), x.dtype),
        scratch_shapes=[
            pltpu.VMEM((S, D, B), x.dtype),
            pltpu.VMEM((2 * S, D // 2, B), x.dtype),
            pltpu.VMEM((D,), g.dtype),
            pltpu.VMEM((D,), b.dtype),
            pltpu.VMEM((D, D), w.dtype),
            pltpu.VMEM((5, D, T), F32),
            pltpu.VMEM((16, D // 4, T), U32),
            pltpu.VMEM((2, D // 2, T), F32),
            pltpu.VMEM((2, 30, HT // 2, T), U32),
            pltpu.VMEM((8, D // 2, T), F32),
            pltpu.VMEM((2, 2, 8, UNIT), F32),
            pltpu.VMEM((2, 8, UNIT), F32),
            pltpu.SemaphoreType.DMA(()),
        ],
        compiler_params=pltpu.CompilerParams(
            vmem_limit_bytes=100 * 2**20,
            flags={"XLA_TPU_RESCHEDULE_DMA_DONES": True},
        ),
    )(jnp.transpose(x, (1, 2, 0)), g, b, w)
    return jnp.transpose(out.reshape(S, D, B), (2, 0, 1))
```
